```python
import jax
import jax.numpy as jnp

def _softmax(x, axis=-1):
    return jax.nn.softmax(x, axis=axis)
def _gelu(x):
    return jax.nn.gelu(x, approximate=True)
def _silu(x):
    return jax.nn.silu(x)
def _sigmoid(x):
    return jax.nn.sigmoid(x)
def _layernorm(x, axis=-1, eps=1e-5):
    m = jnp.mean(x, axis=axis, keepdims=True)
    v = jnp.var(x, axis=axis, keepdims=True)
    return (x - m) / jnp.sqrt(v + eps)
def _scatter_add(tgt, idx, src, axis=0):
    return tgt.at[idx].add(src)
def _segment_sum(src, seg, n):
    return jax.ops.segment_sum(src, seg, n)
class _Rng:
    def __init__(self, key):
        self._k = key
    def _next(self):
        self._k, sub = jax.random.split(self._k)
        return sub
    def normal(self, shape):
        return jax.random.normal(self._next(), shape, dtype=jnp.bfloat16)
    def randint(self, lo, hi, shape):
        return jax.random.randint(self._next(), shape, lo, hi, dtype=jnp.int32)
    def uniform(self, shape, lo=0.0, hi=1.0):
        return jax.random.uniform(self._next(), shape, jnp.bfloat16, lo, hi)
    def permutation(self, n):
        return jax.random.permutation(self._next(), n)


kernel_name = 'gated_mix__sliding_block_cached__glu_gated_swiglu__decode'

def setup_inputs():
    _rng = _Rng(jax.random.key(int.from_bytes(__import__("os").urandom(4), "little")))
    _w = (lambda a: (lambda t: t.astype(jnp.bfloat16) if jnp.issubdtype(t.dtype, jnp.floating) else t)(jnp.asarray(a)))
    def _A_setup():
        B, Sq, D = 1, 1, 640
        Hq, Hkv, Sk, Dh = 32, 32, 32768, 192
        assert Hq % Hkv == 0, (Hq, Hkv)
        return {
            "x": _w((lambda *s: _rng.normal(s) * 0.05)(B, Sq, D)),
            "k_cache": _w((lambda *s: _rng.normal(s) * 0.05)(B, Hkv, Sk, Dh)),
            "v_cache": _w((lambda *s: _rng.normal(s) * 0.05)(B, Hkv, Sk, Dh)),
            "wq": _w((lambda *s: _rng.normal(s) * 0.05)(D, Hq * Dh) * (D ** -0.5)),
            "wo": _w((lambda *s: _rng.normal(s) * 0.05)(Hq * Dh, D) * ((Hq * Dh) ** -0.5)),
        }
    _A_in = _A_setup()

    def _B_setup():
        B, S, D, F = 1, 1, 640, 1536
        return {
            "x": _w((lambda *s: _rng.normal(s) * 0.05)(B, S, D)),
            "w1": _w((lambda *s: _rng.normal(s) * 0.05)(D, F) * (2.0 / D) ** 0.5),
            "w3": _w((lambda *s: _rng.normal(s) * 0.05)(D, F) * (2.0 / D) ** 0.5),
            "w2": _w((lambda *s: _rng.normal(s) * 0.05)(F, D) * (2.0 / F) ** 0.5),
        }
    _B_in = _B_setup()

    return {
        "A_x": _A_in["x"],
        "A_k_cache": _A_in["k_cache"],
        "A_v_cache": _A_in["v_cache"],
        "A_wq": _A_in["wq"],
        "A_wo": _A_in["wo"],
        "B_x": _B_in["x"],
        "B_w1": _B_in["w1"],
        "B_w3": _B_in["w3"],
        "B_w2": _B_in["w2"],
        "gate_w": _w((lambda *s: _rng.normal(s) * 0.05)(640)),
    }

def reference(A_x, A_k_cache, A_v_cache, A_wq, A_wo, B_x, B_w1, B_w3, B_w2, gate_w):
    def _A_ref(x, k_cache, v_cache, wq, wo):
        B, Sq, D = x.shape
        Hq, Dh = 32, 192
        Hkv, Sk = k_cache.shape[1], k_cache.shape[2]
        W = min(4096, max(256, Sk // 4))
        rep = Hq // Hkv
        q = (lambda x, *d: x.transpose(*d))((x @ wq).reshape(B, Sq, Hq, Dh), 0, 2, 1, 3)
        k = jnp.repeat(k_cache[:, :, Sk - W:, :], rep, axis=1)
        v = jnp.repeat(v_cache[:, :, Sk - W:, :], rep, axis=1)
        scores = jnp.einsum("bhqd,bhkd->bhqk", q, k) * (Dh ** -0.5)
        p = _softmax(scores, axis=-1)
        o = jnp.einsum("bhqk,bhkd->bhqd", p, v)
        return (lambda x, *d: x.transpose(*d))(o, 0, 2, 1, 3).reshape(B, Sq, Hq * Dh) @ wo

    def _B_ref(x, w1, w3, w2):
        gate = jnp.einsum("bsd,df->bsf", x, w1)
        up = jnp.einsum("bsd,df->bsf", x, w3)
        h = _silu(gate) * up
        out = jnp.einsum("bsf,fd->bsd", h, w2)
        return out

    x = A_x
    g = _sigmoid((x * gate_w).sum(-1, keepdims=True))
    a = _A_ref(x, A_k_cache, A_v_cache, A_wq, A_wo)
    b = _B_ref(x, B_w1, B_w3, B_w2)
    return g * a + (1 - g) * b
```

```python
import functools

import jax
import jax.numpy as jnp
from jax import lax
import jax.experimental.pallas as pl
import jax.experimental.pallas.tpu as pltpu

_HQ, _DH = 32, 192
_G = 2
_NB = 2
_M = 8
_W2_CHUNKS = 3


def _kernel(x_hbm, k_hbm, v_hbm, wq_hbm, wo_hbm, w1_hbm, w3_hbm, w2_hbm, gw_hbm, o_hbm,
            kb, vb, wqb, wob, w1b, w3b, w2b, xb, gwb, ob, sk, sv, sq, so, sm,
            *, win):
    f32, bf16 = jnp.float32, jnp.bfloat16
    D = xb.shape[-1]
    F = w1b.shape[-1]
    SK = k_hbm.shape[-1]
    GD = _G * _DH
    NG = _HQ // _G
    NB, M = _NB, _M
    FC = F // _W2_CHUNKS

    def rows(g):
        return pl.ds(pl.multiple_of(g * GD, GD), GD)

    def k_cp(g, slot):
        return pltpu.make_async_copy(k_hbm.at[rows(g), pl.ds(SK - win, win)], kb.at[slot], sk.at[slot])

    def v_cp(g, slot):
        return pltpu.make_async_copy(v_hbm.at[rows(g), pl.ds(SK - win, win)], vb.at[slot], sv.at[slot])

    def q_cp(g, slot):
        return pltpu.make_async_copy(wq_hbm.at[:, rows(g)], wqb.at[slot], sq.at[slot])

    def o_cp(g, slot):
        return pltpu.make_async_copy(wo_hbm.at[rows(g), :], wob.at[slot], so.at[slot])

    w1_cp = pltpu.make_async_copy(w1_hbm, w1b, sm.at[0])
    w3_cp = pltpu.make_async_copy(w3_hbm, w3b, sm.at[1])
    w2_cps = [pltpu.make_async_copy(w2_hbm.at[pl.ds(j * FC, FC), :], w2b.at[pl.ds(j * FC, FC), :], sm.at[2 + j])
              for j in range(_W2_CHUNKS)]
    x_cp = pltpu.make_async_copy(x_hbm, xb, sm.at[2 + _W2_CHUNKS])
    g_cp = pltpu.make_async_copy(gw_hbm, gwb, sm.at[3 + _W2_CHUNKS])

    x_cp.start()
    g_cp.start()
    for s in range(NB):
        q_cp(s, s).start()
        k_cp(s, s).start()
        v_cp(s, s).start()
        o_cp(s, s).start()

    x_cp.wait()
    x = xb[...]
    xm = jnp.broadcast_to(x, (M, D))
    row = lax.broadcasted_iota(jnp.int32, (M, GD), 0)
    col = lax.broadcasted_iota(jnp.int32, (M, GD), 1)
    mask = (col >= row * _DH) & (col < (row + 1) * _DH)

    def pair(g, slot, acc, issue_next):
        q_cp(g, slot).wait()
        q = jnp.dot(xm, wqb[slot], preferred_element_type=f32)
        issue_next(0)
        qbd = jnp.where(mask, q, 0.0).astype(bf16)
        k_cp(g, slot).wait()
        s = jnp.dot(qbd, kb[slot], preferred_element_type=f32) * (_DH ** -0.5)
        issue_next(1)
        m = jnp.max(s, axis=-1, keepdims=True)
        p = jnp.exp(s - m)
        l = jnp.sum(p, axis=-1, keepdims=True)
        v_cp(g, slot).wait()
        o = lax.dot_general(p.astype(bf16), vb[slot], (((1,), (1,)), ((), ())),
                            preferred_element_type=f32)
        issue_next(2)
        o = jnp.where(mask, o / l, 0.0).astype(bf16)
        o_cp(g, slot).wait()
        acc = acc + jnp.dot(o, wob[slot], preferred_element_type=f32)
        issue_next(3)
        return acc

    def body(g, acc):
        slot = lax.rem(g, NB)

        def issue_next(which):
            (q_cp, k_cp, v_cp, o_cp)[which](g + NB, slot).start()

        return pair(g, slot, acc, issue_next)

    acc = lax.fori_loop(0, NG - NB, body, jnp.zeros((M, D), f32))

    tail = [w1_cp, w3_cp] + w2_cps
    issued = [0]

    def issue_tail(n=1):
        for _ in range(n):
            if issued[0] < len(tail):
                tail[issued[0]].start()
                issued[0] += 1

    for j in range(NB):
        g = NG - NB + j

        def issue_next(which, j=j):
            if j > 0 or which == 3 and NB == 1:
                issue_tail(len(tail))
            elif which > 0:
                issue_tail()

        acc = pair(g, g % NB, acc, issue_next)
    issue_tail(len(tail))

    a = jnp.sum(acc, axis=0, keepdims=True)
    g_cp.wait()
    gate = jax.nn.sigmoid(jnp.sum(x.astype(f32) * gwb[...].astype(f32).reshape(1, D),
                                  axis=-1, keepdims=True))
    w1_cp.wait()
    gt = jnp.dot(xm, w1b[...], preferred_element_type=f32)
    w3_cp.wait()
    up = jnp.dot(xm, w3b[...], preferred_element_type=f32)
    h = (gt * jax.nn.sigmoid(gt) * up).astype(bf16)
    b = None
    for j in range(_W2_CHUNKS):
        w2_cps[j].wait()
        c = jnp.dot(h[:, j * FC:(j + 1) * FC], w2b[pl.ds(j * FC, FC), :], preferred_element_type=f32)
        b = c if b is None else b + c
    ob[...] = (gate * a + (1 - gate) * b[0:1]).astype(ob.dtype)
    pltpu.sync_copy(ob, o_hbm)


@jax.jit
def pallas_gated_mix__sliding_block_cached__glu_gated_swiglu__decode_kernel(
    A_x: jax.Array,
    A_k_cache: jax.Array,
    A_v_cache: jax.Array,
    A_wq: jax.Array,
    A_wo: jax.Array,
    B_x: jax.Array,
    B_w1: jax.Array,
    B_w3: jax.Array,
    B_w2: jax.Array,
    gate_w: jax.Array,
):
    B, Sq, D = A_x.shape
    _, Hkv, Sk, Dh = A_k_cache.shape
    F = B_w1.shape[1]
    assert (B, Sq, Hkv, Dh) == (1, 1, _HQ, _DH)
    win = min(4096, max(256, Sk // 4))
    GD = _G * _DH
    bf16 = jnp.bfloat16

    kT = jnp.swapaxes(A_k_cache, 2, 3).reshape(Hkv * Dh, Sk)
    vT = jnp.swapaxes(A_v_cache, 2, 3).reshape(Hkv * Dh, Sk)
    x2 = A_x.reshape(1, D)

    any_spec = pl.BlockSpec(memory_space=pl.ANY)
    out = pl.pallas_call(
        functools.partial(_kernel, win=win),
        in_specs=[any_spec] * 9,
        out_specs=any_spec,
        out_shape=jax.ShapeDtypeStruct((1, D), A_x.dtype),
        scratch_shapes=[
            pltpu.VMEM((_NB, GD, win), bf16), pltpu.VMEM((_NB, GD, win), bf16),
            pltpu.VMEM((_NB, D, GD), bf16), pltpu.VMEM((_NB, GD, D), bf16),
            pltpu.VMEM((D, F), bf16), pltpu.VMEM((D, F), bf16), pltpu.VMEM((F, D), bf16),
            pltpu.VMEM((1, D), bf16), pltpu.VMEM((D,), bf16), pltpu.VMEM((1, D), bf16),
            pltpu.SemaphoreType.DMA((_NB,)), pltpu.SemaphoreType.DMA((_NB,)),
            pltpu.SemaphoreType.DMA((_NB,)), pltpu.SemaphoreType.DMA((_NB,)),
            pltpu.SemaphoreType.DMA((4 + _W2_CHUNKS,)),
        ],
        compiler_params=pltpu.CompilerParams(vmem_limit_bytes=100 * 1024 * 1024),
    )(x2, kT, vT, A_wq, A_wo, B_w1, B_w3, B_w2, gate_w)
    return out.reshape(B, Sq, D)
```

```python
import functools

import jax
import jax.numpy as jnp
from jax import lax
import jax.experimental.pallas as pl
import jax.experimental.pallas.tpu as pltpu

_HQ, _DH = 32, 192
_G = 2
_M = 8
_LANE, _RG = 128, 16
_KV_ROWS = 192
_WQ_NB, _WO_NB, _W1_NB = 5, 4, 4
_Q0_K, _Q0_V_WO, _Q0_V_W1, _Q0_V = 10, 6, 6, 16
_W2_CHUNKS = (512, 512, 512)
_H_STEP = 6


def _merge(a, b):
    out, ia, ib = [], 0, 0
    while ia < len(a) or ib < len(b):
        if ib < len(b) and (ia >= len(a) or (ib + 0.5) * len(a) <= (ia + 0.5) * len(b)):
            out.append(b[ib])
            ib += 1
        else:
            out.append(a[ia])
            ia += 1
    return out


def _halves(rows, cols, nr, nc):
    rc = [(r, c) for r in range(0, rows, nr) for c in range(0, cols, nc)]
    h = (len(rc) + 1) // 2
    out = []
    for i in range(h):
        out.append(rc[i] + (0,))
        if i + h < len(rc):
            out.append(rc[i + h] + (1,))
    return out


def _kernel(x_hbm, k_hbm, v_hbm, wq_hbm, wo_hbm, w1_hbm, w3_hbm, w2_hbm, gw_hbm, o_hbm,
            kb, vb, wqb, wob, w1b, w3b, w2b, xb, gwb, ob, sgb, sk, sv, sq, so, sm, *, win):
    f32, bf16 = jnp.float32, jnp.bfloat16
    D = xb.shape[-1]
    F = w3b.shape[-1]
    SK = k_hbm.shape[-1]
    GD = _G * _DH
    NG = _HQ // _G
    M = _M
    nct = win // _LANE
    wq_rows, w1_rows = D // _WQ_NB, D // _W1_NB
    w2off = [sum(_W2_CHUNKS[:i]) for i in range(len(_W2_CHUNKS))]
    nw2 = len(_W2_CHUNKS)

    def build(kv_tag, weights, n0):
        q0, q1 = [], []
        for r in range(0, GD, _KV_ROWS):
            q1 += [(kv_tag, r, c * _LANE) for c in range(nct - n0)]
            q0 += [(kv_tag, r, c * _LANE) for c in range(nct - n0, nct)]
        return _merge([p + (1,) for p in q1], [p + (0,) for p in weights + q0])

    wq_p = [("q", r, c) for r in range(0, wq_rows, _RG) for c in range(0, GD, _LANE)]
    wo_p = [("o", r, c) for r in range(0, GD, _RG) for c in range(0, D, _LANE)]
    w1_p = [("w1", r, c) for r in range(0, w1_rows, _RG) for c in range(0, F, _LANE)]
    list_k = build("k", wq_p, _Q0_K)
    list_v_wo = build("v", wo_p, _Q0_V_WO)
    list_v_w1 = build("v", w1_p, _Q0_V_W1)
    list_v = build("v", [], _Q0_V)

    def off(g):
        return g * GD if isinstance(g, int) else pl.multiple_of(g * GD, GD)

    def issue(pieces, j):
        o = off(j)
        for tag, r, c, queue in pieces:
            if tag == "k":
                cp = pltpu.make_async_copy(k_hbm.at[pl.ds(o + r, _KV_ROWS), pl.ds(SK - win + c, _LANE)],
                                           kb.at[pl.ds(r, _KV_ROWS), pl.ds(c, _LANE)], sk)
            elif tag == "v":
                cp = pltpu.make_async_copy(v_hbm.at[pl.ds(o + r, _KV_ROWS), pl.ds(SK - win + c, _LANE)],
                                           vb.at[pl.ds(r, _KV_ROWS), pl.ds(c, _LANE)], sv)
            elif tag == "q":
                cp = pltpu.make_async_copy(wq_hbm.at[:, pl.ds(r, _RG), pl.ds(o + c, _LANE)],
                                           wqb.at[:, pl.ds(r, _RG), pl.ds(c, _LANE)], sq)
            elif tag == "o":
                cp = pltpu.make_async_copy(wo_hbm.at[:, pl.ds(o + r, _RG), pl.ds(c, _LANE)],
                                           wob.at[:, pl.ds(o + r, _RG), pl.ds(c, _LANE)], so.at[j])
            else:
                cp = pltpu.make_async_copy(w1_hbm.at[:, pl.ds(r, _RG), pl.ds(c, _LANE)],
                                           w1b.at[:, pl.ds(r, _RG), pl.ds(c, _LANE)], sm.at[0])
            cp.start(priority=queue)

    def issue_ffn_tail():
        for r, c, queue in _halves(D, F, _LANE, _LANE):
            pltpu.make_async_copy(w3_hbm.at[pl.ds(r, _LANE), pl.ds(c, _LANE)],
                                  w3b.at[pl.ds(r, _LANE), pl.ds(c, _LANE)], sm.at[1]).start(priority=queue)
        for i in range(nw2):
            for r, c, queue in _halves(_W2_CHUNKS[i], D, _LANE, _LANE):
                pltpu.make_async_copy(w2_hbm.at[pl.ds(w2off[i] + r, _LANE), pl.ds(c, _LANE)],
                                      w2b.at[pl.ds(w2off[i] + r, _LANE), pl.ds(c, _LANE)],
                                      sm.at[2 + i]).start(priority=queue)

    def wait(filled, sem):
        pltpu.make_async_copy(filled, filled, sem).wait()

    def when(cond, fn):
        if isinstance(cond, bool):
            if cond:
                fn()
        else:
            pl.when(cond)(fn)

    x_cp = pltpu.make_async_copy(x_hbm, xb, sm.at[2 + nw2])
    g_cp = pltpu.make_async_copy(gw_hbm, gwb, sm.at[3 + nw2])
    x_cp.start()
    g_cp.start()
    issue(list_k, 0)
    issue(list_v_wo, 0)

    x_cp.wait()
    x = xb[...]
    xm = jnp.broadcast_to(x, (M, D))
    row = lax.broadcasted_iota(jnp.int32, (M, GD), 0)
    col = lax.broadcasted_iota(jnp.int32, (M, GD), 1)
    own = (col >= row * _DH) & (col < (row + 1) * _DH)

    def pair(g, acc):
        j = g + 1
        wait(wqb, sq)
        q = jnp.dot(xm, wqb[...].reshape(D, GD), preferred_element_type=f32)
        qbd = jnp.where(own, q, 0.0).astype(bf16)
        wait(kb, sk)
        s = jnp.dot(qbd, kb[...], preferred_element_type=f32) * (_DH ** -0.5)
        when(j < NG, lambda: issue(list_k, j))
        when(j == NG, issue_ffn_tail)
        m = jnp.max(s, axis=-1, keepdims=True)
        p = jnp.exp(s - m)
        l = jnp.sum(p, axis=-1, keepdims=True)
        wait(vb, sv)
        o = lax.dot_general(p.astype(bf16), vb[...], (((1,), (1,)), ((), ())),
                            preferred_element_type=f32)
        when(j < _WO_NB, lambda: issue(list_v_wo, j))
        when(j == _WO_NB, lambda: issue(list_v_w1, j))
        when((j > _WO_NB) & (j < NG), lambda: issue(list_v, j))
        o = jnp.where(own, o / l, 0.0).astype(bf16)
        when(g < _WO_NB, lambda: wait(wob.at[:, pl.ds(off(g), GD), :], so.at[g]))
        blk = g // _WO_NB
        wo_g = wob[blk, pl.ds(pl.multiple_of((g - blk * _WO_NB) * GD, GD), GD), :]
        acc = acc + jnp.dot(o, wo_g, preferred_element_type=f32)

        def ffn_gate():
            wait(w1b, sm.at[0])
            gt = jnp.dot(xm, w1b[...].reshape(D, F), preferred_element_type=f32)
            sgb[...] = gt * jax.nn.sigmoid(gt)

        when(g == _H_STEP, ffn_gate)
        return acc

    acc = lax.fori_loop(0, NG - 1, pair, jnp.zeros((M, D), f32))
    acc = pair(NG - 1, acc)

    a = jnp.sum(acc, axis=0, keepdims=True)
    g_cp.wait()
    gate = jax.nn.sigmoid(jnp.sum(x.astype(f32) * gwb[...].astype(f32).reshape(1, D),
                                  axis=-1, keepdims=True))
    wait(w3b, sm.at[1])
    up = jnp.dot(xm, w3b[...], preferred_element_type=f32)
    h = (sgb[...] * up).astype(bf16)
    b = None
    for i in range(nw2):
        w2i = w2b.at[pl.ds(w2off[i], _W2_CHUNKS[i]), :]
        wait(w2i, sm.at[2 + i])
        c = jnp.dot(h[:, w2off[i]:w2off[i] + _W2_CHUNKS[i]], w2i[...], preferred_element_type=f32)
        b = c if b is None else b + c
    ob[...] = (gate * a + (1 - gate) * b[0:1]).astype(ob.dtype)
    pltpu.sync_copy(ob, o_hbm)


@jax.jit
def pallas_gated_mix__sliding_block_cached__glu_gated_swiglu__decode_kernel(
    A_x: jax.Array,
    A_k_cache: jax.Array,
    A_v_cache: jax.Array,
    A_wq: jax.Array,
    A_wo: jax.Array,
    B_x: jax.Array,
    B_w1: jax.Array,
    B_w3: jax.Array,
    B_w2: jax.Array,
    gate_w: jax.Array,
):
    B, Sq, D = A_x.shape
    _, Hkv, Sk, Dh = A_k_cache.shape
    F = B_w1.shape[1]
    assert (B, Sq, Hkv, Dh) == (1, 1, _HQ, _DH)
    win = min(4096, max(256, Sk // 4))
    GD = _G * _DH
    bf16 = jnp.bfloat16

    kT = jnp.swapaxes(A_k_cache, 2, 3).reshape(Hkv * Dh, Sk)
    vT = jnp.swapaxes(A_v_cache, 2, 3).reshape(Hkv * Dh, Sk)
    x2 = A_x.reshape(1, D)
    wq3 = A_wq.reshape(_WQ_NB, D // _WQ_NB, Hkv * Dh)
    wo3 = A_wo.reshape(_WO_NB, Hkv * Dh // _WO_NB, D)
    w13 = B_w1.reshape(_W1_NB, D // _W1_NB, F)

    any_spec = pl.BlockSpec(memory_space=pl.ANY)
    out = pl.pallas_call(
        functools.partial(_kernel, win=win),
        in_specs=[any_spec] * 9,
        out_specs=any_spec,
        out_shape=jax.ShapeDtypeStruct((1, D), A_x.dtype),
        scratch_shapes=[
            pltpu.VMEM((GD, win), bf16), pltpu.VMEM((GD, win), bf16),
            pltpu.VMEM(wq3.shape[:2] + (GD,), bf16), pltpu.VMEM(wo3.shape, bf16),
            pltpu.VMEM(w13.shape, bf16), pltpu.VMEM((D, F), bf16), pltpu.VMEM((F, D), bf16),
            pltpu.VMEM((1, D), bf16), pltpu.VMEM((D,), bf16), pltpu.VMEM((1, D), bf16),
            pltpu.VMEM((_M, F), jnp.float32),
            pltpu.SemaphoreType.DMA, pltpu.SemaphoreType.DMA, pltpu.SemaphoreType.DMA,
            pltpu.SemaphoreType.DMA((_WO_NB,)), pltpu.SemaphoreType.DMA((4 + len(_W2_CHUNKS),)),
        ],
        compiler_params=pltpu.CompilerParams(vmem_limit_bytes=64 * 1024 * 1024,
                                             disable_bounds_checks=True,
                                             disable_semaphore_checks=True),
    )(x2, kT, vT, wq3, wo3, w13, B_w3, B_w2, gate_w)
    return out.reshape(B, Sq, D)
```

```python
import functools

import jax
import jax.numpy as jnp
from jax import lax
import jax.experimental.pallas as pl
import jax.experimental.pallas.tpu as pltpu

_HQ, _DH = 32, 192
_G = 2
_M = 8
_LANE, _RG = 128, 16
_KV_ROWS = 96
_WQ_NB, _WO_NB, _W1_NB = 20, 4, 4
_Q0_K, _Q0_V_WO, _Q0_V_W1, _Q0_V = 12, 6, 6, 12
_W2_CHUNKS = (256,) * 6
_H_STEP = 6


def _merge(a, b):
    out, ia, ib = [], 0, 0
    while ia < len(a) or ib < len(b):
        if ib < len(b) and (ia >= len(a) or (ib + 0.5) * len(a) <= (ia + 0.5) * len(b)):
            out.append(b[ib])
            ib += 1
        else:
            out.append(a[ia])
            ia += 1
    return out


def _halves(rows, cols, nr, nc):
    rc = [(r, c) for r in range(0, rows, nr) for c in range(0, cols, nc)]
    h = (len(rc) + 1) // 2
    out = []
    for i in range(h):
        out.append(rc[i] + (0,))
        if i + h < len(rc):
            out.append(rc[i + h] + (1,))
    return out


def _kernel(x_hbm, k_hbm, v_hbm, wq_hbm, wo_hbm, w1_hbm, w3_hbm, w2_hbm, gw_hbm, o_hbm,
            kb, vb, wqb, wob, w1b, w3b, w2b, xb, gwb, ob, sgb, sk, sv, sq, so, sm, *, win):
    f32, bf16 = jnp.float32, jnp.bfloat16
    D = xb.shape[-1]
    F = w3b.shape[-1]
    SK = k_hbm.shape[-1]
    GD = _G * _DH
    NG = _HQ // _G
    M = _M
    nct = win // _LANE
    wq_rows, w1_rows = D // _WQ_NB, D // _W1_NB
    w2off = [sum(_W2_CHUNKS[:i]) for i in range(len(_W2_CHUNKS))]
    nw2 = len(_W2_CHUNKS)

    def build(kv_tag, weights, n0):
        q0, q1 = [], []
        for r in range(0, GD, _KV_ROWS):
            q1 += [(kv_tag, r, c * _LANE) for c in range(nct - n0)]
            q0 += [(kv_tag, r, c * _LANE) for c in range(nct - n0, nct)]
        return _merge([p + (1,) for p in q1], [p + (0,) for p in weights + q0])

    wq_p = [("q", r, c) for r in range(0, wq_rows, _RG) for c in range(0, GD, _LANE)]
    wo_p = [("o", r, c) for r in range(0, GD, _RG) for c in range(0, D, _LANE)]
    w1_p = [("w1", r, c) for r in range(0, w1_rows, _RG) for c in range(0, F, _LANE)]
    list_k = build("k", wq_p, _Q0_K)
    list_v_wo = build("v", wo_p, _Q0_V_WO)
    list_v_w1 = build("v", w1_p, _Q0_V_W1)
    list_v = build("v", [], _Q0_V)

    def off(g):
        return g * GD if isinstance(g, int) else pl.multiple_of(g * GD, GD)

    def issue(pieces, j):
        o = off(j)
        for tag, r, c, queue in pieces:
            if tag == "k":
                cp = pltpu.make_async_copy(k_hbm.at[pl.ds(o + r, _KV_ROWS), pl.ds(SK - win + c, _LANE)],
                                           kb.at[pl.ds(r, _KV_ROWS), pl.ds(c, _LANE)], sk)
            elif tag == "v":
                cp = pltpu.make_async_copy(v_hbm.at[pl.ds(o + r, _KV_ROWS), pl.ds(SK - win + c, _LANE)],
                                           vb.at[pl.ds(r, _KV_ROWS), pl.ds(c, _LANE)], sv)
            elif tag == "q":
                cp = pltpu.make_async_copy(wq_hbm.at[:, pl.ds(r, _RG), pl.ds(o + c, _LANE)],
                                           wqb.at[:, pl.ds(r, _RG), pl.ds(c, _LANE)], sq)
            elif tag == "o":
                cp = pltpu.make_async_copy(wo_hbm.at[:, pl.ds(o + r, _RG), pl.ds(c, _LANE)],
                                           wob.at[:, pl.ds(o + r, _RG), pl.ds(c, _LANE)], so.at[j])
            else:
                cp = pltpu.make_async_copy(w1_hbm.at[:, pl.ds(r, _RG), pl.ds(c, _LANE)],
                                           w1b.at[:, pl.ds(r, _RG), pl.ds(c, _LANE)], sm.at[0])
            cp.start(priority=queue)

    def issue_ffn_tail():
        for r, c, queue in _halves(D, F, _LANE, _LANE):
            pltpu.make_async_copy(w3_hbm.at[pl.ds(r, _LANE), pl.ds(c, _LANE)],
                                  w3b.at[pl.ds(r, _LANE), pl.ds(c, _LANE)], sm.at[1]).start(priority=queue)
        for i in range(nw2):
            for r, c, queue in _halves(_W2_CHUNKS[i], D, _LANE, _LANE):
                pltpu.make_async_copy(w2_hbm.at[pl.ds(w2off[i] + r, _LANE), pl.ds(c, _LANE)],
                                      w2b.at[pl.ds(w2off[i] + r, _LANE), pl.ds(c, _LANE)],
                                      sm.at[2 + i]).start(priority=queue)

    def wait(filled, sem):
        pltpu.make_async_copy(filled, filled, sem).wait()

    def when(cond, fn):
        if isinstance(cond, bool):
            if cond:
                fn()
        else:
            pl.when(cond)(fn)

    x_cp = pltpu.make_async_copy(x_hbm, xb, sm.at[2 + nw2])
    g_cp = pltpu.make_async_copy(gw_hbm, gwb, sm.at[3 + nw2])
    x_cp.start()
    g_cp.start()
    issue(list_k, 0)
    issue(list_v_wo, 0)

    x_cp.wait()
    x = xb[...]
    xm = jnp.broadcast_to(x, (M, D))
    row = lax.broadcasted_iota(jnp.int32, (M, GD), 0)
    col = lax.broadcasted_iota(jnp.int32, (M, GD), 1)
    own = (col >= row * _DH) & (col < (row + 1) * _DH)

    def pair(g, acc, last=False):
        j = g + 1
        wait(wqb, sq)
        q = jnp.dot(xm, wqb[...].reshape(D, GD), preferred_element_type=f32)
        qbd = jnp.where(own, q, 0.0).astype(bf16)
        wait(kb, sk)
        s = jnp.dot(qbd, kb[...], preferred_element_type=f32) * (_DH ** -0.5)
        if last:
            issue_ffn_tail()
        else:
            issue(list_k, j)
        m = jnp.max(s, axis=-1, keepdims=True)
        p = jnp.exp(s - m)
        l = jnp.sum(p, axis=-1, keepdims=True)
        wait(vb, sv)
        o = lax.dot_general(p.astype(bf16), vb[...], (((1,), (1,)), ((), ())),
                            preferred_element_type=f32)
        if not last:
            when(j < _WO_NB, lambda: issue(list_v_wo, j))
            when(j == _WO_NB, lambda: issue(list_v_w1, j))
            when(j > _WO_NB, lambda: issue(list_v, j))
        o = jnp.where(own, o / l, 0.0).astype(bf16)
        when(g < _WO_NB, lambda: wait(wob.at[:, pl.ds(off(g), GD), :], so.at[g]))
        blk = g // _WO_NB
        wo_g = wob[blk, pl.ds(pl.multiple_of((g - blk * _WO_NB) * GD, GD), GD), :]
        acc = acc + jnp.dot(o, wo_g, preferred_element_type=f32)

        def ffn_gate():
            wait(w1b, sm.at[0])
            gt = jnp.dot(xm, w1b[...].reshape(D, F), preferred_element_type=f32)
            sgb[...] = gt * jax.nn.sigmoid(gt)

        when(g == _H_STEP, ffn_gate)
        return acc

    acc = lax.fori_loop(0, NG - 1, pair, jnp.zeros((M, D), f32))
    acc = pair(NG - 1, acc, last=True)

    a = jnp.sum(acc, axis=0, keepdims=True)
    g_cp.wait()
    gate = jax.nn.sigmoid(jnp.sum(x.astype(f32) * gwb[...].astype(f32).reshape(1, D),
                                  axis=-1, keepdims=True))
    wait(w3b, sm.at[1])
    up = jnp.dot(xm, w3b[...], preferred_element_type=f32)
    h = (sgb[...] * up).astype(bf16)
    b = None
    for i in range(nw2):
        w2i = w2b.at[pl.ds(w2off[i], _W2_CHUNKS[i]), :]
        wait(w2i, sm.at[2 + i])
        c = jnp.dot(h[:, w2off[i]:w2off[i] + _W2_CHUNKS[i]], w2i[...], preferred_element_type=f32)
        b = c if b is None else b + c
    ob[...] = (gate * a + (1 - gate) * b[0:1]).astype(ob.dtype)
    pltpu.sync_copy(ob, o_hbm)


@jax.jit
def pallas_gated_mix__sliding_block_cached__glu_gated_swiglu__decode_kernel(
    A_x: jax.Array,
    A_k_cache: jax.Array,
    A_v_cache: jax.Array,
    A_wq: jax.Array,
    A_wo: jax.Array,
    B_x: jax.Array,
    B_w1: jax.Array,
    B_w3: jax.Array,
    B_w2: jax.Array,
    gate_w: jax.Array,
):
    B, Sq, D = A_x.shape
    _, Hkv, Sk, Dh = A_k_cache.shape
    F = B_w1.shape[1]
    assert (B, Sq, Hkv, Dh) == (1, 1, _HQ, _DH)
    win = min(4096, max(256, Sk // 4))
    GD = _G * _DH
    bf16 = jnp.bfloat16

    kT = jnp.swapaxes(A_k_cache, 2, 3).reshape(Hkv * Dh, Sk)
    vT = jnp.swapaxes(A_v_cache, 2, 3).reshape(Hkv * Dh, Sk)
    x2 = A_x.reshape(1, D)
    wq3 = A_wq.reshape(_WQ_NB, D // _WQ_NB, Hkv * Dh)
    wo3 = A_wo.reshape(_WO_NB, Hkv * Dh // _WO_NB, D)
    w13 = B_w1.reshape(_W1_NB, D // _W1_NB, F)

    any_spec = pl.BlockSpec(memory_space=pl.ANY)
    out = pl.pallas_call(
        functools.partial(_kernel, win=win),
        in_specs=[any_spec] * 9,
        out_specs=any_spec,
        out_shape=jax.ShapeDtypeStruct((1, D), A_x.dtype),
        scratch_shapes=[
            pltpu.VMEM((GD, win), bf16), pltpu.VMEM((GD, win), bf16),
            pltpu.VMEM(wq3.shape[:2] + (GD,), bf16), pltpu.VMEM(wo3.shape, bf16),
            pltpu.VMEM(w13.shape, bf16), pltpu.VMEM((D, F), bf16), pltpu.VMEM((F, D), bf16),
            pltpu.VMEM((1, D), bf16), pltpu.VMEM((D,), bf16), pltpu.VMEM((1, D), bf16),
            pltpu.VMEM((_M, F), jnp.float32),
            pltpu.SemaphoreType.DMA, pltpu.SemaphoreType.DMA, pltpu.SemaphoreType.DMA,
            pltpu.SemaphoreType.DMA((_WO_NB,)), pltpu.SemaphoreType.DMA((4 + len(_W2_CHUNKS),)),
        ],
        compiler_params=pltpu.CompilerParams(vmem_limit_bytes=64 * 1024 * 1024,
                                             disable_semaphore_checks=True),
    )(x2, kT, vT, wq3, wo3, w13, B_w3, B_w2, gate_w)
    return out.reshape(B, Sq, D)
```

```python
import functools

import jax
import jax.numpy as jnp
from jax import lax
import jax.experimental.pallas as pl
import jax.experimental.pallas.tpu as pltpu

_HQ, _DH = 32, 192
_G = 2
_M = 8
_LANE, _RG = 128, 16
_KV_ROWS = 96
_WQ_NB, _WO_NB, _W1_NB = 20, 4, 4
_Q0_K, _Q0_V_WO, _Q0_V_W1, _Q0_V = 12, 6, 6, 12
_W2_CHUNKS = (256,) * 6
_H_STEP = 6


def _merge(a, b):
    out, ia, ib = [], 0, 0
    while ia < len(a) or ib < len(b):
        if ib < len(b) and (ia >= len(a) or (ib + 0.5) * len(a) <= (ia + 0.5) * len(b)):
            out.append(b[ib])
            ib += 1
        else:
            out.append(a[ia])
            ia += 1
    return out


def _halves(rows, cols, nr, nc, col_major=False):
    rc = [(r, c) for r in range(0, rows, nr) for c in range(0, cols, nc)]
    if col_major:
        rc.sort(key=lambda p: (p[1], p[0]))
    h = (len(rc) + 1) // 2
    out = []
    for i in range(h):
        out.append(rc[i] + (0,))
        if i + h < len(rc):
            out.append(rc[i + h] + (1,))
    return out


def _kernel(x_hbm, k_hbm, v_hbm, wq_hbm, wo_hbm, w1_hbm, w3_hbm, w2_hbm, gw_hbm, o_hbm,
            kb, vb, wqb, wob, w1b, w3b, w2b, xb, gwb, ob, sgb, sk, sv, sq, so, sm, *, win):
    f32, bf16 = jnp.float32, jnp.bfloat16
    D = xb.shape[-1]
    F = w3b.shape[-1]
    SK = k_hbm.shape[-1]
    GD = _G * _DH
    NG = _HQ // _G
    M = _M
    nct = win // _LANE
    wq_rows, w1_rows = D // _WQ_NB, D // _W1_NB
    w2off = [sum(_W2_CHUNKS[:i]) for i in range(len(_W2_CHUNKS))]
    nw2 = len(_W2_CHUNKS)

    def build(kv_tag, weights, n0):
        q0, q1 = [], []
        for r in range(0, GD, _KV_ROWS):
            q1 += [(kv_tag, r, c * _LANE) for c in range(nct - n0)]
            q0 += [(kv_tag, r, c * _LANE) for c in range(nct - n0, nct)]
        return _merge([p + (1,) for p in q1], [p + (0,) for p in weights + q0])

    wq_p = [("q", r, c) for r in range(0, wq_rows, _RG) for c in range(0, GD, _LANE)]
    wo_p = [("o", r, c) for r in range(0, GD, _RG) for c in range(0, D, _LANE)]
    w1_p = [("w1", r, c) for r in range(0, w1_rows, _RG) for c in range(0, F, _LANE)]
    list_k = build("k", wq_p, _Q0_K)
    list_v_wo = build("v", wo_p, _Q0_V_WO)
    list_v_w1 = build("v", w1_p, _Q0_V_W1)
    list_v = build("v", [], _Q0_V)

    def off(g):
        return g * GD if isinstance(g, int) else pl.multiple_of(g * GD, GD)

    def issue(pieces, j):
        o = off(j)
        for tag, r, c, queue in pieces:
            if tag == "k":
                cp = pltpu.make_async_copy(k_hbm.at[pl.ds(o + r, _KV_ROWS), pl.ds(SK - win + c, _LANE)],
                                           kb.at[pl.ds(r, _KV_ROWS), pl.ds(c, _LANE)], sk)
            elif tag == "v":
                cp = pltpu.make_async_copy(v_hbm.at[pl.ds(o + r, _KV_ROWS), pl.ds(SK - win + c, _LANE)],
                                           vb.at[pl.ds(r, _KV_ROWS), pl.ds(c, _LANE)], sv)
            elif tag == "q":
                cp = pltpu.make_async_copy(wq_hbm.at[:, pl.ds(r, _RG), pl.ds(o + c, _LANE)],
                                           wqb.at[:, pl.ds(r, _RG), pl.ds(c, _LANE)], sq)
            elif tag == "o":
                cp = pltpu.make_async_copy(wo_hbm.at[:, pl.ds(o + r, _RG), pl.ds(c, _LANE)],
                                           wob.at[:, pl.ds(o + r, _RG), pl.ds(c, _LANE)], so.at[j])
            else:
                cp = pltpu.make_async_copy(w1_hbm.at[:, pl.ds(r, _RG), pl.ds(c, _LANE)],
                                           w1b.at[:, pl.ds(r, _RG), pl.ds(c, _LANE)], sm.at[0])
            cp.start(priority=queue)

    def issue_ffn_tail():
        for r, c, queue in _halves(D, F, D // 2, _LANE, col_major=True):
            pltpu.make_async_copy(w3_hbm.at[pl.ds(r, D // 2), pl.ds(c, _LANE)],
                                  w3b.at[pl.ds(r, D // 2), pl.ds(c, _LANE)], sm.at[1]).start(priority=queue)
        for i in range(nw2):
            for r, c, queue in _halves(_W2_CHUNKS[i], D, _LANE, _LANE):
                pltpu.make_async_copy(w2_hbm.at[pl.ds(w2off[i] + r, _LANE), pl.ds(c, _LANE)],
                                      w2b.at[pl.ds(w2off[i] + r, _LANE), pl.ds(c, _LANE)],
                                      sm.at[2 + i]).start(priority=queue)

    def wait(filled, sem):
        pltpu.make_async_copy(filled, filled, sem).wait()

    def when(cond, fn):
        if isinstance(cond, bool):
            if cond:
                fn()
        else:
            pl.when(cond)(fn)

    x_cp = pltpu.make_async_copy(x_hbm, xb, sm.at[2 + nw2])
    g_cp = pltpu.make_async_copy(gw_hbm, gwb, sm.at[3 + nw2])
    x_cp.start()
    g_cp.start()
    issue(list_k, 0)
    issue(list_v_wo, 0)

    x_cp.wait()
    x = xb[...]
    xm = jnp.broadcast_to(x, (M, D))
    row = lax.broadcasted_iota(jnp.int32, (M, GD), 0)
    col = lax.broadcasted_iota(jnp.int32, (M, GD), 1)
    own = (col >= row * _DH) & (col < (row + 1) * _DH)

    def pair(g, acc, last=False):
        j = g + 1
        wait(wqb, sq)
        q = jnp.dot(xm, wqb[...].reshape(D, GD), preferred_element_type=f32)
        qbd = jnp.where(own, q, 0.0).astype(bf16)
        wait(kb, sk)
        s = jnp.dot(qbd, kb[...], preferred_element_type=f32) * (_DH ** -0.5)
        if last:
            issue_ffn_tail()
        else:
            issue(list_k, j)
        m = jnp.max(s, axis=-1, keepdims=True)
        p = jnp.exp(s - m)
        l = jnp.sum(p, axis=-1, keepdims=True)
        wait(vb, sv)
        o = lax.dot_general(p.astype(bf16), vb[...], (((1,), (1,)), ((), ())),
                            preferred_element_type=f32)
        if not last:
            when(j < _WO_NB, lambda: issue(list_v_wo, j))
            when(j == _WO_NB, lambda: issue(list_v_w1, j))
            when(j > _WO_NB, lambda: issue(list_v, j))
        o = jnp.where(own, o / l, 0.0).astype(bf16)
        when(g < _WO_NB, lambda: wait(wob.at[:, pl.ds(off(g), GD), :], so.at[g]))
        blk = g // _WO_NB
        wo_g = wob[blk, pl.ds(pl.multiple_of((g - blk * _WO_NB) * GD, GD), GD), :]
        acc = acc + jnp.dot(o, wo_g, preferred_element_type=f32)

        def ffn_gate():
            wait(w1b, sm.at[0])
            gt = jnp.dot(xm, w1b[...].reshape(D, F), preferred_element_type=f32)
            sgb[...] = gt * jax.nn.sigmoid(gt)

        when(g == _H_STEP, ffn_gate)
        return acc

    acc = lax.fori_loop(0, NG - 1, pair, jnp.zeros((M, D), f32))
    acc = pair(NG - 1, acc, last=True)

    a = jnp.sum(acc, axis=0, keepdims=True)
    g_cp.wait()
    gate = jax.nn.sigmoid(jnp.sum(x.astype(f32) * gwb[...].astype(f32).reshape(1, D),
                                  axis=-1, keepdims=True))
    wait(w3b, sm.at[1])
    up = jnp.dot(xm, w3b[...], preferred_element_type=f32)
    h = (sgb[...] * up).astype(bf16)
    b = None
    for i in range(nw2):
        w2i = w2b.at[pl.ds(w2off[i], _W2_CHUNKS[i]), :]
        wait(w2i, sm.at[2 + i])
        c = jnp.dot(h[:, w2off[i]:w2off[i] + _W2_CHUNKS[i]], w2i[...], preferred_element_type=f32)
        b = c if b is None else b + c
    ob[...] = (gate * a + (1 - gate) * b[0:1]).astype(ob.dtype)
    pltpu.sync_copy(ob, o_hbm)


@jax.jit
def pallas_gated_mix__sliding_block_cached__glu_gated_swiglu__decode_kernel(
    A_x: jax.Array,
    A_k_cache: jax.Array,
    A_v_cache: jax.Array,
    A_wq: jax.Array,
    A_wo: jax.Array,
    B_x: jax.Array,
    B_w1: jax.Array,
    B_w3: jax.Array,
    B_w2: jax.Array,
    gate_w: jax.Array,
):
    B, Sq, D = A_x.shape
    _, Hkv, Sk, Dh = A_k_cache.shape
    F = B_w1.shape[1]
    assert (B, Sq, Hkv, Dh) == (1, 1, _HQ, _DH)
    win = min(4096, max(256, Sk // 4))
    GD = _G * _DH
    bf16 = jnp.bfloat16

    kT = jnp.swapaxes(A_k_cache, 2, 3).reshape(Hkv * Dh, Sk)
    vT = jnp.swapaxes(A_v_cache, 2, 3).reshape(Hkv * Dh, Sk)
    x2 = A_x.reshape(1, D)
    wq3 = A_wq.reshape(_WQ_NB, D // _WQ_NB, Hkv * Dh)
    wo3 = A_wo.reshape(_WO_NB, Hkv * Dh // _WO_NB, D)
    w13 = B_w1.reshape(_W1_NB, D // _W1_NB, F)

    any_spec = pl.BlockSpec(memory_space=pl.ANY)
    out = pl.pallas_call(
        functools.partial(_kernel, win=win),
        in_specs=[any_spec] * 9,
        out_specs=any_spec,
        out_shape=jax.ShapeDtypeStruct((1, D), A_x.dtype),
        scratch_shapes=[
            pltpu.VMEM((GD, win), bf16), pltpu.VMEM((GD, win), bf16),
            pltpu.VMEM(wq3.shape[:2] + (GD,), bf16), pltpu.VMEM(wo3.shape, bf16),
            pltpu.VMEM(w13.shape, bf16), pltpu.VMEM((D, F), bf16), pltpu.VMEM((F, D), bf16),
            pltpu.VMEM((1, D), bf16), pltpu.VMEM((D,), bf16), pltpu.VMEM((1, D), bf16),
            pltpu.VMEM((_M, F), jnp.float32),
            pltpu.SemaphoreType.DMA, pltpu.SemaphoreType.DMA, pltpu.SemaphoreType.DMA,
            pltpu.SemaphoreType.DMA((_WO_NB,)), pltpu.SemaphoreType.DMA((4 + len(_W2_CHUNKS),)),
        ],
        compiler_params=pltpu.CompilerParams(vmem_limit_bytes=64 * 1024 * 1024,
                                             disable_semaphore_checks=True),
    )(x2, kT, vT, wq3, wo3, w13, B_w3, B_w2, gate_w)
    return out.reshape(B, Sq, D)
```
